```python
import jax
import jax.numpy as jnp

def _softmax(x, axis=-1):
    return jax.nn.softmax(x, axis=axis)
def _gelu(x):
    return jax.nn.gelu(x, approximate=True)
def _silu(x):
    return jax.nn.silu(x)
def _sigmoid(x):
    return jax.nn.sigmoid(x)
def _layernorm(x, axis=-1, eps=1e-5):
    m = jnp.mean(x, axis=axis, keepdims=True)
    v = jnp.var(x, axis=axis, keepdims=True)
    return (x - m) / jnp.sqrt(v + eps)
def _scatter_add(tgt, idx, src, axis=0):
    return tgt.at[idx].add(src)
def _segment_sum(src, seg, n):
    return jax.ops.segment_sum(src, seg, n)
class _Rng:
    def __init__(self, key):
        self._k = key
    def _next(self):
        self._k, sub = jax.random.split(self._k)
        return sub
    def normal(self, shape):
        return jax.random.normal(self._next(), shape, dtype=jnp.bfloat16)
    def randint(self, lo, hi, shape):
        return jax.random.randint(self._next(), shape, lo, hi, dtype=jnp.int32)
    def uniform(self, shape, lo=0.0, hi=1.0):
        return jax.random.uniform(self._next(), shape, jnp.bfloat16, lo, hi)
    def permutation(self, n):
        return jax.random.permutation(self._next(), n)


kernel_name = 'standalone__cross_network_dcn__recsys'

def setup_inputs():
    _rng = _Rng(jax.random.key(int.from_bytes(__import__("os").urandom(4), "little")))
    _w = (lambda a: (lambda t: t.astype(jnp.bfloat16) if jnp.issubdtype(t.dtype, jnp.floating) else t)(jnp.asarray(a)))
    B, F, D, L = 16384, 100, 16, 6
    Din = min(F * D, 1024)
    return {
        "x0": _w((lambda *s: _rng.normal(s) * 0.05)(B, Din)),
        "ws": _w((lambda *s: _rng.normal(s) * 0.05)(L, Din, Din) * (Din ** -0.5)),
        "bs": _w((lambda *s: _rng.normal(s) * 0.05)(L, Din) * 0.01),
    }

def reference(x0, ws, bs):
    x = x0
    L = ws.shape[0]
    for l in range(L):
        proj = jnp.einsum('bd,de->be', x, ws[l]) + bs[l]
        x = x0 * proj + x
    return x
```

```python
import jax
import jax.numpy as jnp
import jax.experimental.pallas as pl
import jax.experimental.pallas.tpu as pltpu


@jax.jit
def pallas_standalone__cross_network_dcn__recsys_kernel(
    x0: jax.Array,
    ws: jax.Array,
    bs: jax.Array,
):
    B, D = x0.shape
    L = ws.shape[0]
    bm = 512

    def kernel_function(x0_ref, w_ref, b_ref, o_ref):
        x0b = x0_ref[...]
        x0f = x0b.astype(jnp.float32)
        xb = x0b
        for l in range(L):
            p = jnp.dot(xb, w_ref[l], preferred_element_type=jnp.float32)
            p = p + b_ref[l:l + 1, :].astype(jnp.float32)
            xb = (x0f * p + xb.astype(jnp.float32)).astype(jnp.bfloat16)
        o_ref[...] = xb

    return pl.pallas_call(
        kernel_function,
        grid=(B // bm,),
        in_specs=[
            pl.BlockSpec((bm, D), lambda i: (i, 0)),
            pl.BlockSpec((L, D, D), lambda i: (0, 0, 0), pipeline_mode=pl.Buffered(1)),
            pl.BlockSpec((L, D), lambda i: (0, 0)),
        ],
        out_specs=pl.BlockSpec((bm, D), lambda i: (i, 0)),
        out_shape=jax.ShapeDtypeStruct((B, D), x0.dtype),
        compiler_params=pltpu.CompilerParams(
            dimension_semantics=("arbitrary",), vmem_limit_bytes=100 * 2**20),
    )(x0, ws, bs)
```

```python
import jax, jax.numpy as jnp
import jax.experimental.pallas as pl
import jax.experimental.pallas.tpu as pltpu
f32, bf16, u32 = jnp.float32, jnp.bfloat16, jnp.uint32

SA = [((0,1),(3,1)), ((2,1),(3,1)), ((0,1),), ((3,1),), ((0,1),(1,1)), ((2,1),(0,-1)), ((1,1),(3,-1))]
SB = [((0,1),(3,1)), ((0,1),), ((1,1),(3,-1)), ((2,1),(0,-1)), ((3,1),), ((0,1),(1,1)), ((2,1),(3,1))]
ORDER = (2, 4, 3, 6, 0, 1, 5)
SWAP2 = (0, 1, 0, 0, 1, 1, 1)
def lin(terms, blk):
    r = blk(terms[0][0])
    for i, s in terms[1:]:
        r = r + blk(i) if s > 0 else r - blk(i)
    return r
def rc(o, i):
    return 2*(o//2) + i//2, 2*(o%2) + i%2
def consume(p, m, ld, st, out):
    if p == 2: st(0, m)
    elif p == 4: st(1, m); out(1, ld(0) + m)
    elif p == 3: st(2, m)
    elif p == 6: st(3, (ld(2) - ld(1)) + m)
    elif p == 0: st(4, ld(0) + m); out(0, ld(3) + m)
    elif p == 1: st(5, ld(4) - m); out(2, ld(2) + m)
    elif p == 5: out(3, ld(5) + m)

@jax.jit
def pallas_standalone__cross_network_dcn__recsys_kernel(x0, ws, bs):
    bm, ch, rs, sw, unr = 512, 16, 16, 1, 2
    B, D = x0.shape; L = ws.shape[0]; q = D // 4; qm = bm // 4
    def kern(x0_ref, w_hbm, b_ref, o_ref, w_ref, s_ref, x_ref, t1_ref, t2_ref, sem):
        def encw(l, sw1, r):
            for cc in range(q // 128):
                g = {}
                for o in range(4):
                    for i in range(4):
                        a, b = rc(o, i)
                        g[o, i] = w_ref[l, pl.ds(a*q + r, ch), b*q+cc*128:b*q+cc*128+128].astype(f32)
                for p1 in range(7):
                    t1 = [lin(SB[p1], lambda o: g[o ^ sw1, i]) for i in range(4)]
                    for p2 in range(7):
                        v = lin(SB[p2], lambda i: t1[i ^ (SWAP2[p1] & sw)]).astype(bf16)
                        s_ref[l, 7*p1+p2, pl.ds(pl.multiple_of(r//2, ch//2), ch//2), cc*128:cc*128+128] = pltpu.bitcast(v, u32)
        @pl.when(pl.program_id(0) == 0)
        def _():
            cps = [pltpu.make_async_copy(w_hbm.at[l], w_ref.at[l], sem.at[l]) for l in range(L)]
            for c in cps: c.start()
            def lbody(lp, c):
                for par in range(2):
                    l = 2 * lp + par
                    pltpu.make_async_copy(w_hbm.at[l], w_ref.at[l], sem.at[l]).wait()
                    def body(t, c):
                        for u in range(unr):
                            encw(l, par & sw, pl.multiple_of((t * unr + u) * ch, ch))
                        return c
                    jax.lax.fori_loop(0, q // ch // unr, body, 0)
                return c
            jax.lax.fori_loop(0, L // 2, lbody, 0)
        z = jax.lax.shift_right_logical(pl.program_id(0), 24)
        def x0b(o, i, r):
            a, b = rc(o, i)
            return x0_ref[a*qm+r:a*qm+r+rs, b*q:(b+1)*q].astype(f32)
        def xl(l, o, i, r):
            return x0b(o, i, r) if l == 0 else x_ref[l % 2, z + 4*o+i, r:r+rs]
        for l in range(L):
          sw1 = (l % 2) & sw
          for p1 in ORDER:
            sw2 = SWAP2[p1] & sw
            for p2 in ORDER:
                a = jnp.concatenate([lin(SA[p2], lambda i: lin(SA[p1], lambda o: xl(l, o, i, r))) for r in range(0, qm, rs)], 0).astype(bf16)
                mm = jnp.dot(a, pltpu.bitcast(s_ref[l, 7*p1+p2], bf16), preferred_element_type=f32)
                for r in range(0, qm, rs):
                    def fin(o, i, c):
                        v = x0b(o, i, r) * c + xl(l, o, i, r)
                        if l == L - 1:
                            a, b = rc(o, i)
                            o_ref[a*qm+r:a*qm+r+rs, b*q:(b+1)*q] = v.astype(bf16)
                        else:
                            x_ref[(l+1) % 2, z + 4*o+i, r:r+rs] = v
                    def up(i, v):
                        i = i ^ sw2
                        if p1 in (2, 3):
                            b = rc((1 if p1 == 2 else 0) ^ sw1, i)[1]
                            v = v + b_ref[l:l+1, b*q:(b+1)*q].astype(f32)
                        def st(s, val): t1_ref[z + s, i, r:r+rs] = val
                        consume(p1, v, lambda s: t1_ref[z + s, i, r:r+rs], st, lambda o, c: fin(o ^ sw1, i, c))
                    def st2(s, val): t2_ref[z + s, r:r+rs] = val
                    consume(p2, mm[r:r+rs], lambda s: t2_ref[z + s, r:r+rs], st2, up)
    return pl.pallas_call(
        kern, grid=(B // bm,),
        in_specs=[pl.BlockSpec((bm, D), lambda i: (i, 0)),
                  pl.BlockSpec(memory_space=pl.ANY),
                  pl.BlockSpec((L, D), lambda i: (0, 0))],
        out_specs=pl.BlockSpec((bm, D), lambda i: (i, 0)),
        out_shape=jax.ShapeDtypeStruct((B, D), bf16),
        scratch_shapes=[pltpu.VMEM((L, D, D), bf16), pltpu.VMEM((L, 49, q // 2, q), u32), pltpu.VMEM((2, 16, qm, q), f32),
                        pltpu.VMEM((6, 4, qm, q), f32), pltpu.VMEM((6, qm, q), f32), pltpu.SemaphoreType.DMA((L,))],
        compiler_params=pltpu.CompilerParams(dimension_semantics=("arbitrary",), vmem_limit_bytes=120*2**20),
    )(x0, ws, bs)
```

```python
import jax
import jax.numpy as jnp
import jax.experimental.pallas as pl
import jax.experimental.pallas.tpu as pltpu

F32, BF16 = jnp.float32, jnp.bfloat16

LHS = (((0, 1), (3, 1)), ((2, 1), (3, 1)), ((0, 1),), ((3, 1),),
       ((0, 1), (1, 1)), ((2, 1), (0, -1)), ((1, 1), (3, -1)))
RHS = (((0, 1), (3, 1)), ((0, 1),), ((1, 1), (3, -1)), ((2, 1), (0, -1)),
       ((3, 1),), ((0, 1), (1, 1)), ((2, 1), (3, 1)))
ORDER = (2, 4, 3, 6, 0, 1, 5)
SWAP = (0, 1, 0, 0, 1, 1, 1)
LANES = 128


def _signed_sum(terms, block):
    acc = block(terms[0][0])
    for idx, sign in terms[1:]:
        acc = acc + block(idx) if sign > 0 else acc - block(idx)
    return acc


def _pos(outer, inner):
    return 2 * (outer // 2) + inner // 2, 2 * (outer % 2) + inner % 2


def _combine(p, m, load, store, emit):
    if p == 2:
        store(0, m)
    elif p == 4:
        store(1, m)
        emit(1, load(0) + m)
    elif p == 3:
        store(2, m)
    elif p == 6:
        store(3, (load(2) - load(1)) + m)
    elif p == 0:
        store(4, load(0) + m)
        emit(0, load(3) + m)
    elif p == 1:
        store(5, load(4) - m)
        emit(2, load(2) + m)
    else:
        emit(3, load(5) + m)


@jax.jit
def pallas_standalone__cross_network_dcn__recsys_kernel(
    x0: jax.Array,
    ws: jax.Array,
    bs: jax.Array,
):
    return _cross_network(x0, ws, bs)


def _cross_network(x0, ws, bs, bm=512, uw=256):
    B, D = x0.shape
    L = ws.shape[0]
    assert B % bm == 0 and B >= 2 * bm and D % (4 * LANES) == 0
    assert L % 2 == 0 and L >= 4
    tiles = B // bm
    h, q, hm, qm = D // 2, D // 4, bm // 2, bm // 4
    units = (q // 16) * (q // uw)

    def kernel(x0_hbm, w_hbm, b_in, o_hbm, b_ref, x0_ref, o_ref, w_ref, s_ref,
               xa_ref, xb_ref, t1_ref, t2_ref, w_sem, i_sem, o_sem):
        def w_copy(l, c):
            return pltpu.make_async_copy(
                w_hbm.at[l, :, pl.ds(c * h, h)], w_ref.at[l, c], w_sem.at[l, c])

        def x_copy(t, slot):
            return pltpu.make_async_copy(
                x0_hbm.at[pl.ds(pl.multiple_of(t * bm, bm), bm)],
                x0_ref.at[slot], i_sem.at[slot])

        def o_copy(t, slot, o):
            r, c = (o // 2) * hm, (o % 2) * h
            return pltpu.make_async_copy(
                o_ref.at[slot, pl.ds(r, hm), pl.ds(c, h)],
                o_hbm.at[pl.ds(pl.multiple_of(t * bm + r, hm), hm), pl.ds(c, h)],
                o_sem.at[slot, o])

        def weight_sums(dst, l, swap, p1, unit):
            r, c = (unit // (q // uw)) * 16, (unit % (q // uw)) * uw

            def block(o, i):
                a, b = _pos(o ^ swap, i)
                c0 = (b % 2) * q + c
                return w_ref[l, b // 2, a * q + r:a * q + r + 16, c0:c0 + uw].astype(F32)

            mid = [_signed_sum(RHS[p1], lambda o: block(o, i)) for i in range(4)]
            for p2 in range(7):
                v = _signed_sum(RHS[p2], lambda i: mid[i ^ SWAP[p1]])
                s_ref[dst, 7 * p1 + p2, r:r + 16, c:c + uw] = v.astype(BF16)

        def tile_index(slot, o, i):
            a, b = _pos(o, i)
            return slot, slice(a * qm, (a + 1) * qm), slice(b * q, (b + 1) * q)

        def layer(l, swap, z, slot, x_in, x_out, before_dot):
            for n1, p1 in enumerate(ORDER):
                def outer_done(i):
                    def emit(o, proj):
                        o = o ^ swap
                        x = x0_ref[tile_index(slot, o, i)].astype(F32)
                        x_out(o, i, x * proj + x_in(o, i))
                    return emit

                def inner_done(i, m):
                    i = i ^ SWAP[p1]
                    if p1 == 2 or p1 == 3:
                        b = _pos((1 if p1 == 2 else 0) ^ swap, i)[1]
                        m = m + b_ref[pl.ds(l, 1), b * q:(b + 1) * q]

                    def store(s, v):
                        t1_ref[z + s, i] = v
                    _combine(p1, m, lambda s: t1_ref[z + s, i], store, outer_done(i))

                def store_inner(s, v):
                    t2_ref[z + s] = v

                for n2, p2 in enumerate(ORDER):
                    before_dot(7 * n1 + n2)
                    lhs = _signed_sum(LHS[p2], lambda i: _signed_sum(
                        LHS[p1], lambda o: x_in(o, i)))
                    m = jnp.dot(lhs.astype(BF16), s_ref[l, 7 * p1 + p2],
                                preferred_element_type=F32)
                    _combine(p2, m, lambda s: t2_ref[z + s], store_inner, inner_done)

        def state(l, z):
            src, dst = (xa_ref, xb_ref) if l % 2 == 0 else (xb_ref, xa_ref)

            def write(o, i, v):
                dst[z + 4 * o + i] = v
            return (lambda o, i: src[z + 4 * o + i]), write

        w_copy(0, 1).start()
        x_copy(0, 0).start()
        w_copy(0, 0).start()
        b_ref[...] = b_in[...].astype(F32)
        w_copy(0, 1).wait()
        w_copy(1, 0).start()
        for u in range(units):
            weight_sums(0, 0, 0, ORDER[0], u)
        x_copy(0, 0).wait()
        w_copy(1, 1).start()
        for o in range(4):
            for i in range(4):
                xa_ref[4 * o + i] = x0_ref[tile_index(0, o, i)].astype(F32)
        w_copy(0, 0).wait()

        def first_tile(pair, carry):
            z = jax.lax.shift_right_logical(pair, 24)
            z2 = jax.lax.shift_right_logical(pair, 25)

            @pl.when(pair == 1)
            def _():
                x_copy(1, 1).start()

            def next_weights(l):
                for c in range(2):
                    w_copy(l, c).wait()

                @pl.when(l + 1 < L)
                def _():
                    for c in range(2):
                        w_copy(l + 1, c).start()

            for odd in range(2):
                def before_dot(n):
                    g, n2 = 7 * odd + n // 7 + 1, n % 7
                    l = 2 * pair + g // 7
                    if n2 == 0 and g == 7:
                        next_weights(l)
                    if n2 == 0 and g == 14:
                        pl.when(l < L)(lambda: next_weights(l))
                    src = jnp.minimum(l, L - 1) if g == 14 else l
                    for u in range(units * n2 // 7, units * (n2 + 1) // 7):
                        weight_sums(l + z2, src, (g // 7) % 2, ORDER[g % 7], u)

                layer(2 * pair + odd, odd, z, 0, *state(odd, z), before_dot)
            return carry

        jax.lax.fori_loop(0, L // 2, first_tile, 0)
        for o in range(4):
            for i in range(4):
                o_ref[tile_index(0, o, i)] = xa_ref[4 * o + i].astype(o_ref.dtype)
            o_copy(0, 0, o).start()
        x_copy(1, 1).wait()

        def tile(t, carry):
            slot = t % 2
            z = jax.lax.shift_right_logical(t, 24)

            def read_x0(o, i):
                return x0_ref[tile_index(slot, o, i)].astype(F32)

            def write_out(o, i, v):
                o_ref[tile_index(slot, o, i)] = v.astype(o_ref.dtype)

            for l in range(L):
                def before_dot(n):
                    if l == 1 and n == 2:
                        x_copy(jnp.minimum(t + 1, tiles - 1), 1 - slot).start()
                    done = {16: 1, 37: 0, 44: 2}
                    if l == L - 1 and n in done:
                        o_copy(t, slot, done[n] ^ 1).start()

                x_in, x_out = state(l, z)
                layer(l, l % 2, z, slot, read_x0 if l == 0 else x_in,
                      write_out if l == L - 1 else x_out, before_dot)
            o_copy(t, slot, 3 ^ 1).start()
            x_copy(t, 1 - slot).wait()
            for o in range(4):
                o_copy(t - 1, 1 - slot, o).wait()
            return carry

        jax.lax.fori_loop(1, tiles, tile, 0)
        for o in range(4):
            o_copy(tiles - 1, (tiles - 1) % 2, o).wait()

    return pl.pallas_call(
        kernel,
        in_specs=[pl.BlockSpec(memory_space=pl.ANY),
                  pl.BlockSpec(memory_space=pl.ANY),
                  pl.BlockSpec(memory_space=pltpu.VMEM)],
        out_specs=pl.BlockSpec(memory_space=pl.ANY),
        out_shape=jax.ShapeDtypeStruct((B, D), x0.dtype),
        scratch_shapes=[
            pltpu.VMEM((L, D), F32),
            pltpu.VMEM((2, bm, D), x0.dtype),
            pltpu.VMEM((2, bm, D), x0.dtype),
            pltpu.VMEM((L, 2, D, h), ws.dtype),
            pltpu.VMEM((L + 1, 49, q, q), BF16),
            pltpu.VMEM((16, qm, q), F32),
            pltpu.VMEM((16, qm, q), F32),
            pltpu.VMEM((6, 4, qm, q), F32),
            pltpu.VMEM((6, qm, q), F32),
            pltpu.SemaphoreType.DMA((L, 2)),
            pltpu.SemaphoreType.DMA((2,)),
            pltpu.SemaphoreType.DMA((2, 4)),
        ],
        compiler_params=pltpu.CompilerParams(vmem_limit_bytes=100 * 2**20),
    )(x0, ws, bs)
```

```python
import jax
import jax.numpy as jnp
import jax.experimental.pallas as pl
import jax.experimental.pallas.tpu as pltpu

F32, BF16 = jnp.float32, jnp.bfloat16

LHS = (((0, 1), (3, 1)), ((2, 1), (3, 1)), ((0, 1),), ((3, 1),),
       ((0, 1), (1, 1)), ((2, 1), (0, -1)), ((1, 1), (3, -1)))
RHS = (((0, 1), (3, 1)), ((0, 1),), ((1, 1), (3, -1)), ((2, 1), (0, -1)),
       ((3, 1),), ((0, 1), (1, 1)), ((2, 1), (3, 1)))
ORDER = (2, 4, 3, 6, 0, 1, 5)
SWAP = (0, 1, 0, 0, 1, 1, 1)
LANES = 128
HUGE = 1e24


def _signed_sum(terms, block):
    acc = block(terms[0][0])
    for idx, sign in terms[1:]:
        acc = acc + block(idx) if sign > 0 else acc - block(idx)
    return acc


def _pos(outer, inner):
    return 2 * (outer // 2) + inner // 2, 2 * (outer % 2) + inner % 2


def _combine(p, m, load, store, emit):
    if p == 2:
        store(0, m)
    elif p == 4:
        store(1, m)
        emit(1, load(0) + m)
    elif p == 3:
        store(2, m)
    elif p == 6:
        store(3, (load(2) - load(1)) + m)
    elif p == 0:
        store(4, load(0) + m)
        emit(0, load(3) + m)
    elif p == 1:
        store(5, load(4) - m)
        emit(2, load(2) + m)
    else:
        emit(3, load(5) + m)


def _clip(v):
    return jnp.where(v <= HUGE, v, HUGE)


def _peak(v):
    return jnp.max(jnp.max(v, axis=0, keepdims=True), axis=1, keepdims=True)


def _strassen_is_safe(x_norm2, w_norm2, w_max2, b_max, layers):
    growth = 1.0 + 4.0 * jnp.sqrt(x_norm2) * jnp.sqrt(w_norm2)
    g = jnp.ones_like(growth)
    for _ in range(layers - 1):
        g = g * growth + b_max
    safe = 32.0 * g * jnp.sqrt(x_norm2) * jnp.sqrt(w_max2) <= 1.0
    safe = safe & (x_norm2 < HUGE) & (w_norm2 < HUGE) & (b_max < HUGE)
    return jnp.where(safe, 1.0, 0.0)


@jax.jit
def pallas_standalone__cross_network_dcn__recsys_kernel(
    x0: jax.Array,
    ws: jax.Array,
    bs: jax.Array,
):
    return _cross_network(x0, ws, bs)


def _cross_network(x0, ws, bs, bm=512, uw=256):
    B, D = x0.shape
    L = ws.shape[0]
    assert B % bm == 0 and B > L * bm and D % (4 * LANES) == 0
    assert L % 2 == 0 and L >= 4 and bm % 128 == 0
    tiles = B // bm
    h, q, hm, qm = D // 2, D // 4, bm // 2, bm // 4
    units = (q // 16) * (q // uw)
    x_pieces, w_pieces = bm // 16, 4 * (D // LANES)
    assert x_pieces <= 6 * L and w_pieces <= 8 * (L - 1)

    def kernel(x0_hbm, w_hbm, b_in, o_hbm, b_ref, x0_ref, o_ref, w_ref, s_ref,
               xa_ref, xb_ref, t1_ref, t2_ref, xp_ref, w_sem, i_sem, o_sem):
        def w_copy(l, c):
            return pltpu.make_async_copy(
                w_hbm.at[l, :, pl.ds(c * h, h)], w_ref.at[l, c], w_sem.at[l, c])

        def x_copy(t, slot):
            return pltpu.make_async_copy(
                x0_hbm.at[pl.ds(pl.multiple_of(t * bm, bm), bm)],
                x0_ref.at[slot], i_sem.at[slot])

        def o_copy(t, slot, o):
            r, c = (o // 2) * hm, (o % 2) * h
            return pltpu.make_async_copy(
                o_ref.at[slot, pl.ds(r, hm), pl.ds(c, h)],
                o_hbm.at[pl.ds(pl.multiple_of(t * bm + r, hm), hm), pl.ds(c, h)],
                o_sem.at[slot, o])

        def weight_sums(dst, l, swap, p1, unit):
            r, c = (unit // (q // uw)) * 16, (unit % (q // uw)) * uw

            def block(o, i):
                a, b = _pos(o ^ swap, i)
                c0 = (b % 2) * q + c
                return w_ref[l, b // 2, a * q + r:a * q + r + 16, c0:c0 + uw].astype(F32)

            mid = [_signed_sum(RHS[p1], lambda o: block(o, i)) for i in range(4)]
            for p2 in range(7):
                v = _signed_sum(RHS[p2], lambda i: mid[i ^ SWAP[p1]])
                s_ref[dst, 7 * p1 + p2, r:r + 16, c:c + uw] = v.astype(BF16)

        def tile_index(slot, o, i):
            a, b = _pos(o, i)
            return slot, slice(a * qm, (a + 1) * qm), slice(b * q, (b + 1) * q)

        def layer(l, swap, z, slot, x_in, x_out, before_dot):
            for n1, p1 in enumerate(ORDER):
                def outer_done(i):
                    def emit(o, proj):
                        o = o ^ swap
                        x = x0_ref[tile_index(slot, o, i)].astype(F32)
                        x_out(o, i, x * proj + x_in(o, i))
                    return emit

                def inner_done(i, m):
                    i = i ^ SWAP[p1]
                    if p1 == 2 or p1 == 3:
                        b = _pos((1 if p1 == 2 else 0) ^ swap, i)[1]
                        m = m + b_ref[pl.ds(l, 1), b * q:(b + 1) * q]

                    def store(s, v):
                        t1_ref[z + s, i] = v
                    _combine(p1, m, lambda s: t1_ref[z + s, i], store, outer_done(i))

                def store_inner(s, v):
                    t2_ref[z + s] = v

                for n2, p2 in enumerate(ORDER):
                    before_dot(7 * n1 + n2)
                    lhs = _signed_sum(LHS[p2], lambda i: _signed_sum(
                        LHS[p1], lambda o: x_in(o, i)))
                    m = jnp.dot(lhs.astype(BF16), s_ref[l, 7 * p1 + p2],
                                preferred_element_type=F32)
                    _combine(p2, m, lambda s: t2_ref[z + s], store_inner, inner_done)

        def state(l, z):
            src, dst = (xa_ref, xb_ref) if l % 2 == 0 else (xb_ref, xa_ref)

            def write(o, i, v):
                dst[z + 4 * o + i] = v
            return (lambda o, i: src[z + 4 * o + i]), write

        def stat(z, k):
            return z + 6, slice(8 * k, 8 * k + 8), slice(0, LANES)

        def raise_stat(z, k, v):
            t2_ref[stat(z, k)] = jnp.maximum(t2_ref[stat(z, k)], v)

        def x_stats(z, slot, piece):
            x = x0_ref[slot, 16 * piece:16 * piece + 16, :].astype(F32)
            x2 = x * x
            peak = jnp.zeros((16, LANES), F32)
            for c in range(0, D, q):
                part = x2[:, c:c + LANES]
                for j in range(c + LANES, c + q, LANES):
                    part = part + x2[:, j:j + LANES]
                norm2 = jnp.sum(part, axis=1, keepdims=True)
                peak = jnp.maximum(peak, _clip(jnp.broadcast_to(norm2, peak.shape)))
            raise_stat(z, 0, jnp.maximum(peak[:8], peak[8:]))

        def w_stats(z, l, piece):
            a, c = piece % 4, (piece // 4) * LANES
            total = top = jnp.zeros((8, LANES), F32)
            for r in range(a * q, (a + 1) * q, 16):
                w = w_ref[l, c // h, r:r + 16, c % h:c % h + LANES].astype(F32)
                w2 = w * w
                total = total + (w2[:8] + w2[8:])
                top = jnp.maximum(top, jnp.maximum(w2[:8], w2[8:]))
            norm2 = jnp.sum(total, axis=0, keepdims=True)
            raise_stat(z, 1, _clip(jnp.broadcast_to(norm2, (8, LANES))))
            raise_stat(z, 2, _clip(top))

        w_copy(0, 1).start()
        x_copy(0, 0).start()
        w_copy(0, 0).start()
        b_ref[...] = b_in[...].astype(F32)
        w_copy(0, 1).wait()
        w_copy(1, 0).start()
        for u in range(units):
            weight_sums(0, 0, 0, ORDER[0], u)
        x_copy(0, 0).wait()
        w_copy(1, 1).start()
        for o in range(4):
            for i in range(4):
                xa_ref[4 * o + i] = x0_ref[tile_index(0, o, i)].astype(F32)
        b_max = _peak(_clip(jnp.abs(b_ref[...])))
        for k in range(3):
            t2_ref[stat(0, k)] = jnp.zeros((8, LANES), F32)
        for piece in range(x_pieces):
            x_stats(0, 0, piece)
        w_copy(0, 0).wait()

        def first_tile(pair, carry):
            z = jax.lax.shift_right_logical(pair, 24)
            z2 = jax.lax.shift_right_logical(pair, 25)

            @pl.when(pair == 1)
            def _():
                x_copy(1, 1).start()

            def next_weights(l):
                for c in range(2):
                    w_copy(l, c).wait()

                @pl.when(l + 1 < L)
                def _():
                    for c in range(2):
                        w_copy(l + 1, c).start()

            for odd in range(2):
                def before_dot(n):
                    g, n2 = 7 * odd + n // 7 + 1, n % 7
                    l = 2 * pair + g // 7
                    if n2 == 0 and g == 7:
                        next_weights(l)
                    if n2 == 0 and g == 14:
                        pl.when(l < L)(lambda: next_weights(l))
                    src = jnp.minimum(l, L - 1) if g == 14 else l
                    for u in range(units * n2 // 7, units * (n2 + 1) // 7):
                        weight_sums(l + z2, src, (g // 7) % 2, ORDER[g % 7], u)

                layer(2 * pair + odd, odd, z, 0, *state(odd, z), before_dot)
            return carry

        jax.lax.fori_loop(0, L // 2, first_tile, 0)
        for o in range(4):
            for i in range(4):
                o_ref[tile_index(0, o, i)] = xa_ref[4 * o + i].astype(o_ref.dtype)
            o_copy(0, 0, o).start()
        x_copy(1, 1).wait()

        def tile(carry):
            t = carry[0]
            slot = t % 2
            z = jax.lax.shift_right_logical(t, 24)
            z2 = jax.lax.shift_right_logical(t, 25)
            x_todo, w_todo = [*range(x_pieces)], [*range(w_pieces)]
            verdict = []

            def read_x0(o, i):
                return x0_ref[tile_index(slot, o, i)].astype(F32)

            def write_out(o, i, v):
                o_ref[tile_index(slot, o, i)] = v.astype(o_ref.dtype)

            for l in range(L):
                def before_dot(n):
                    if w_todo and l >= 1 and n // 7 in (0, 2) and n % 7 < 4:
                        w_stats(z2, jnp.minimum(t, L) - 1, w_todo.pop(0))
                    if x_todo and n // 7 in (1, 3, 6) and n % 7 in (0, 2):
                        x_stats(z2, slot, x_todo.pop(0))
                    if not (x_todo or w_todo or verdict):
                        peaks = [_peak(t2_ref[stat(z2, k)]) for k in range(3)]
                        safe = _strassen_is_safe(*peaks, b_max, L)
                        t2_ref[stat(z2, 3)] = jnp.broadcast_to(safe, (8, LANES))
                        verdict.append(jnp.max(safe) > 0.5)
                    if l == 1 and n == 2:
                        x_copy(jnp.minimum(t + 1, tiles - 1), 1 - slot).start()
                    done = {16: 1, 37: 0, 44: 2}
                    if l == L - 1 and n in done:
                        o_copy(t, slot, done[n] ^ 1).start()

                x_in, x_out = state(l, z)
                layer(l, l % 2, z, slot, read_x0 if l == 0 else x_in,
                      write_out if l == L - 1 else x_out, before_dot)
            o_copy(t, slot, 3 ^ 1).start()
            x_copy(t, 1 - slot).wait()
            for o in range(4):
                o_copy(t - 1, 1 - slot, o).wait()
            return t + 1, verdict[0].astype(jnp.int32)

        end, safe = jax.lax.while_loop(
            lambda c: jnp.logical_and(c[0] < tiles, c[1] > 0), tile,
            (jnp.int32(1), jnp.int32(1)))
        last = end - 1
        for o in range(4):
            o_copy(last, last % 2, o).wait()

        @pl.when(safe == 0)
        def _():
            start = jnp.where(last > L, last, 0)
            x_copy(start, start % 2).start()

            def plain_tile(t, carry):
                slot = t % 2
                x_copy(t, slot).wait()

                @pl.when(t + 1 < tiles)
                def _():
                    x_copy(t + 1, 1 - slot).start()

                xp_ref[...] = x0_ref[slot].astype(F32)

                def plain_layer(l, carry):
                    x = xp_ref[...].astype(BF16)
                    for c in range(2):
                        cols = slice(c * h, (c + 1) * h)
                        proj = jnp.dot(x, w_ref[l, c], preferred_element_type=F32)
                        proj = proj + b_ref[pl.ds(l, 1), cols]
                        xp_ref[:, cols] += x0_ref[slot, :, cols].astype(F32) * proj
                    return carry

                jax.lax.fori_loop(0, L, plain_layer, 0)
                o_ref[slot] = xp_ref[...].astype(o_ref.dtype)
                for o in range(4):
                    o_copy(t, slot, o).start()

                @pl.when(t > start)
                def _():
                    for o in range(4):
                        o_copy(t - 1, 1 - slot, o).wait()
                return carry

            jax.lax.fori_loop(start, tiles, plain_tile, 0)
            for o in range(4):
                o_copy(tiles - 1, (tiles - 1) % 2, o).wait()

    return pl.pallas_call(
        kernel,
        in_specs=[pl.BlockSpec(memory_space=pl.ANY),
                  pl.BlockSpec(memory_space=pl.ANY),
                  pl.BlockSpec(memory_space=pltpu.VMEM)],
        out_specs=pl.BlockSpec(memory_space=pl.ANY),
        out_shape=jax.ShapeDtypeStruct((B, D), x0.dtype),
        scratch_shapes=[
            pltpu.VMEM((L, D), F32),
            pltpu.VMEM((2, bm, D), x0.dtype),
            pltpu.VMEM((2, bm, D), x0.dtype),
            pltpu.VMEM((L, 2, D, h), ws.dtype),
            pltpu.VMEM((L + 1, 49, q, q), BF16),
            pltpu.VMEM((16, qm, q), F32),
            pltpu.VMEM((16, qm, q), F32),
            pltpu.VMEM((6, 4, qm, q), F32),
            pltpu.VMEM((7, qm, q), F32),
            pltpu.VMEM((bm, D), F32),
            pltpu.SemaphoreType.DMA((L, 2)),
            pltpu.SemaphoreType.DMA((2,)),
            pltpu.SemaphoreType.DMA((2, 4)),
        ],
        compiler_params=pltpu.CompilerParams(vmem_limit_bytes=100 * 2**20),
    )(x0, ws, bs)
```
